```python
import jax
import jax.numpy as jnp

def _softmax(x, axis=-1):
    return jax.nn.softmax(x, axis=axis)
def _gelu(x):
    return jax.nn.gelu(x, approximate=True)
def _silu(x):
    return jax.nn.silu(x)
def _sigmoid(x):
    return jax.nn.sigmoid(x)
def _layernorm(x, axis=-1, eps=1e-5):
    m = jnp.mean(x, axis=axis, keepdims=True)
    v = jnp.var(x, axis=axis, keepdims=True)
    return (x - m) / jnp.sqrt(v + eps)
def _scatter_add(tgt, idx, src, axis=0):
    return tgt.at[idx].add(src)
def _segment_sum(src, seg, n):
    return jax.ops.segment_sum(src, seg, n)
class _Rng:
    def __init__(self, key):
        self._k = key
    def _next(self):
        self._k, sub = jax.random.split(self._k)
        return sub
    def normal(self, shape):
        return jax.random.normal(self._next(), shape, dtype=jnp.bfloat16)
    def randint(self, lo, hi, shape):
        return jax.random.randint(self._next(), shape, lo, hi, dtype=jnp.int32)
    def uniform(self, shape, lo=0.0, hi=1.0):
        return jax.random.uniform(self._next(), shape, jnp.bfloat16, lo, hi)
    def permutation(self, n):
        return jax.random.permutation(self._next(), n)


kernel_name = 'standalone__gqa_block_cached__near_ridge'

def _fwd_setup_inputs():
    _rng = _Rng(jax.random.key(int.from_bytes(__import__("os").urandom(4), "little")))
    _w = (lambda a: (lambda t: t.astype(jnp.bfloat16) if jnp.issubdtype(t.dtype, jnp.floating) else t)(jnp.asarray(a)))
    B, Sq, D = 16, 64, 640
    Hq, Hkv, Sk, Dh = 32, 32, 512, 192
    assert Hq % Hkv == 0, (Hq, Hkv)
    return {
        "x": _w((lambda *s: _rng.normal(s) * 0.05)(B, Sq, D)),
        "k_cache": _w((lambda *s: _rng.normal(s) * 0.05)(B, Hkv, Sk, Dh)),
        "v_cache": _w((lambda *s: _rng.normal(s) * 0.05)(B, Hkv, Sk, Dh)),
        "wq": _w((lambda *s: _rng.normal(s) * 0.05)(D, Hq * Dh) * (D ** -0.5)),
        "wo": _w((lambda *s: _rng.normal(s) * 0.05)(Hq * Dh, D) * ((Hq * Dh) ** -0.5)),
    }

def _fwd_reference(x, k_cache, v_cache, wq, wo):
    B, Sq, D = x.shape
    Hq, Dh = 32, 192
    Hkv = k_cache.shape[1]
    rep = Hq // Hkv
    q = (lambda x, *d: x.transpose(*d))((x @ wq).reshape(B, Sq, Hq, Dh), 0, 2, 1, 3)
    k = jnp.repeat(k_cache, rep, axis=1)
    v = jnp.repeat(v_cache, rep, axis=1)
    scores = jnp.einsum("bhqd,bhkd->bhqk", q, k) * (Dh ** -0.5)
    p = _softmax(scores, axis=-1)
    o = jnp.einsum("bhqk,bhkd->bhqd", p, v)
    return (lambda x, *d: x.transpose(*d))(o, 0, 2, 1, 3).reshape(B, Sq, Hq * Dh) @ wo


def setup_inputs():
    _inp = _fwd_setup_inputs()
    _gk = jax.random.fold_in(jax.random.key(int.from_bytes(__import__("os").urandom(4), "little")), 2**31 - 1)
    _shapes = [[16, 64, 640]]
    _dtypes = ['bfloat16']
    _gks = jax.random.split(_gk, len(_shapes))
    _gs = [jax.random.normal(k, s, dtype=jnp.dtype(d)) * 0.05 for k, s, d in zip(_gks, _shapes, _dtypes)]
    _inp["grad_out"] = _gs[0]
    return _inp

def reference(x, k_cache, v_cache, wq, wo, grad_out):
    _const = dict()
    def _f(*_d):
        return _fwd_reference(**{'x': _d[0], 'k_cache': _d[1], 'v_cache': _d[2], 'wq': _d[3], 'wo': _d[4], **_const})
    _out, _vjp = jax.vjp(_f, x, k_cache, v_cache, wq, wo)
    _grads = _vjp(grad_out)
    _out0 = jnp.asarray(_out)
    return (_out0, *[jnp.asarray(_g) for _g in _grads])
```

```python
import functools
import jax
import jax.numpy as jnp
from jax import lax
import jax.experimental.pallas as pl
import jax.experimental.pallas.tpu as pltpu

B, SQ, D = 16, 64, 640
H, SK, DH = 32, 512, 192
HP = 2
W = HP * DH
M = B * SQ
NSTEP = H // HP
SCALE = DH ** -0.5
LOG2E = 1.4426950408889634
F32 = jnp.float32
BF16 = jnp.bfloat16
GB = 4
NG = B // GB

NN = (((1,), (0,)), ((), ()))
NT = (((1,), (1,)), ((), ()))
TN = (((0,), (0,)), ((), ()))

def dot(a, b, dn):
    return lax.dot_general(a, b, dn, preferred_element_type=F32)

def pad_pair(y):
    lane = lax.broadcasted_iota(jnp.int32, (y.shape[0], 128), 1)
    mid = y[:, 128:256]
    return jnp.concatenate([y[:, 0:128], jnp.where(lane < 64, mid, 0.0), jnp.where(lane >= 64, mid, 0.0), y[:, 256:384]],
                           axis=1).astype(BF16)

def kernel(x_hbm, g_hbm, wq_hbm, wo_hbm, kt_hbm, vt_hbm,
           out_hbm, dx_hbm, dkt_hbm, dvt_hbm, dwq_hbm, dwo_hbm,
           x_ref, g_ref, wq_buf, wo_buf, kt_buf, vt_buf, dkt_buf, dvt_buf, dwq_buf, dwo_buf, out_buf, dx_buf,
           q_scr, do_scr, o_scr, dq_scr, p_scr, ds_scr, xt_scr, out_acc, dx_acc,
           rsem, wsem, msem, *, unroll, wr, nocompute):
    step = pl.program_id(0)
    slot = step % 2
    last = NSTEP - 1

    def hrows(i):
        return pl.ds(pl.multiple_of(i * W, 128), W)

    def rd_kv(i, g):
        bs = pl.ds(g * GB, GB)
        return [pltpu.make_async_copy(src.at[bs, hrows(i), :], dst.at[i % 2, bs], rsem.at[a * NG + g])
                for a, (src, dst) in enumerate(((kt_hbm, kt_buf), (vt_hbm, vt_buf)))]

    def rd_w(i):
        return [pltpu.make_async_copy(wq_hbm.at[:, hrows(i)], wq_buf.at[i % 2], rsem.at[2 * NG]),
                pltpu.make_async_copy(wo_hbm.at[hrows(i), :], wo_buf.at[i % 2], rsem.at[2 * NG + 1])]

    def wr_kv_start(i, g):
        bs = pl.ds(g * GB, GB)
        for r in range(W // wr):
            for a, (src, dst) in enumerate(((dkt_buf, dkt_hbm), (dvt_buf, dvt_hbm))):
                pltpu.make_async_copy(src.at[i % 2, bs, pl.ds(r * wr, wr), :],
                                      dst.at[bs, pl.ds(pl.multiple_of(i * W + r * wr, 16), wr), :],
                                      wsem.at[a * NG + g]).start()

    def wr_kv_wait(i, g):
        bs = pl.ds(g * GB, GB)
        for a, (src, dst) in enumerate(((dkt_buf, dkt_hbm), (dvt_buf, dvt_hbm))):
            pltpu.make_async_copy(src.at[i % 2, bs], dst.at[bs, hrows(i), :], wsem.at[a * NG + g]).wait()

    def wr_w(i):
        return [pltpu.make_async_copy(dwq_buf.at[i % 2], dwq_hbm.at[:, hrows(i)], wsem.at[2 * NG]),
                pltpu.make_async_copy(dwo_buf.at[i % 2], dwo_hbm.at[hrows(i), :], wsem.at[2 * NG + 1])]

    def start_r(i):
        for c in rd_w(i): c.start()
        for g in range(NG):
            for c in rd_kv(i, g): c.start()

    def wait_r_main(i):
        for c in rd_w(i): c.wait()
        for g in range(NG - 1):
            for c in rd_kv(i, g): c.wait()

    def wait_r_tail(i):
        for c in rd_kv(i, NG - 1): c.wait()

    x_cp = pltpu.make_async_copy(x_hbm, x_ref, msem.at[0])
    g_cp = pltpu.make_async_copy(g_hbm, g_ref, msem.at[1])
    out_cp = pltpu.make_async_copy(out_buf, out_hbm, msem.at[2])
    dx_cp = pltpu.make_async_copy(dx_buf, dx_hbm, msem.at[3])

    @pl.when(step == 0)
    def _():
        x_cp.start()
        g_cp.start()
        start_r(0)
        out_acc[...] = jnp.zeros_like(out_acc)
        dx_acc[...] = jnp.zeros_like(dx_acc)
        x_cp.wait()
        xt_scr[...] = x_ref[...].T
        g_cp.wait()
        for c in rd_w(0): c.wait()

    wq_ref = wq_buf.at[slot]
    wo_ref = wo_buf.at[slot]
    kt_ref = kt_buf.at[slot]
    vt_ref = vt_buf.at[slot]
    dkt_ref = dkt_buf.at[slot]
    dvt_ref = dvt_buf.at[slot]

    if not nocompute:
        q_scr[...] = pad_pair(dot(x_ref[...], wq_ref[...], NN))
        do_scr[...] = pad_pair(dot(g_ref[...], wo_ref[...], NT))

    @pl.when(step == 0)
    def _():
        for g in range(NG - 1):
            for c in rd_kv(0, g): c.wait()

    def rows(b):
        if isinstance(b, int):
            return pl.ds(b * SQ, SQ)
        return pl.ds(pl.multiple_of(b * SQ, SQ), SQ)

    def stage1_mm(b, h):
        r = rows(b)
        s = dot(q_scr[r, h * 256:(h + 1) * 256], kt_ref[b, h * 128:h * 128 + 256, :], NN)
        dp = dot(do_scr[r, h * 256:(h + 1) * 256], vt_ref[b, h * 128:h * 128 + 256, :], NN)
        return s, dp

    def softmax(s, dp):
        m = jnp.max(s, axis=-1, keepdims=True)
        e = jnp.exp2((s - m) * (SCALE * LOG2E))
        l = jnp.sum(e, axis=-1, keepdims=True)
        p = e * (1.0 / l)
        delta = jnp.sum(p * dp, axis=-1, keepdims=True)
        ds = (p * (dp - delta) * SCALE).astype(BF16)
        return p.astype(BF16), ds

    def stage2(b, h, pb, ds):
        r = rows(b)
        lo = 64 * h
        o = dot(pb, vt_ref[b, h * 128:h * 128 + 256, :], NT)
        dq = dot(ds, kt_ref[b, h * 128:h * 128 + 256, :], NT)
        o_scr[r, h * DH:(h + 1) * DH] = o[:, lo:lo + DH].astype(BF16)
        dq_scr[r, h * DH:(h + 1) * DH] = dq[:, lo:lo + DH].astype(BF16)
        dot_ = do_scr[r, h * 256:(h + 1) * 256].T[lo:lo + DH]
        qt_ = q_scr[r, h * 256:(h + 1) * 256].T[lo:lo + DH]
        dvt_ref[b, h * DH:(h + 1) * DH, :] = dot(dot_, pb, NN).astype(BF16)
        dkt_ref[b, h * DH:(h + 1) * DH, :] = dot(qt_, ds, NN).astype(BF16)

    if not nocompute:
        for h in range(HP):
            pb, ds = softmax(*stage1_mm(0, h))
            p_scr[h] = pb
            ds_scr[h] = ds

    @pl.when(step >= 2)
    def _():
        wr_kv_wait(step - 2, NG - 1)
        for c in wr_w(step - 2): c.wait()

    @pl.when(step >= 1)
    def _():
        for g in range(NG - 2):
            wr_kv_wait(step - 1, g)

    wait_r_tail(step)

    @pl.when(step < last)
    def _():
        start_r(step + 1)

    @pl.when(step == last)
    def _():
        wr_kv_start(step - 1, NG - 1)
        for c in wr_w(step - 1): c.start()

    def body(j, c):
        @pl.when(jnp.logical_and(step == last, j >= 2))
        def _():
            @pl.when(j == 4)
            def _():
                wr_kv_wait(step - 1, NG - 2)
            wr_kv_start(step, j - 2)
        if nocompute:
            return c
        cur = [(p_scr[h], ds_scr[h]) for h in range(HP)]
        for u in range(unroll):
            b = j * unroll + u
            nxt = []
            for h in range(HP):
                sdp = stage1_mm(b + 1, h)
                stage2(b, h, *cur[h])
                nxt.append(softmax(*sdp))
            cur = nxt
        for h in range(HP):
            p_scr[h] = cur[h][0]
            ds_scr[h] = cur[h][1]
        return c
    assert unroll == 3
    lax.fori_loop(0, (B - 1) // unroll, body, 0)

    @pl.when(step < last)
    def _():
        wait_r_main(step + 1)
        @pl.when(step >= 1)
        def _():
            wr_kv_wait(step - 1, NG - 2)
            wr_kv_start(step - 1, NG - 1)
            for c in wr_w(step - 1): c.start()
        for g in range(NG - 1):
            wr_kv_start(step, g)

    if not nocompute:
        for h in range(HP):
            stage2(B - 1, h, p_scr[h], ds_scr[h])

    @pl.when(step == last)
    def _():
        wr_kv_wait(step - 1, NG - 1)
        wr_kv_start(step, NG - 1)
        for c in wr_w(step - 1): c.wait()

    if not nocompute:
        o = o_scr[...]
        dq = dq_scr[...]
        out_acc[...] += dot(o, wo_ref[...], NN)
        dx_acc[...] += dot(dq, wq_ref[...], NT)
        dwo_buf[slot] = dot(o, g_ref[...], TN).astype(BF16)
        dwq_buf[slot] = dot(xt_scr[...], dq, NN).astype(BF16)

    @pl.when(step == last)
    def _():
        for c in wr_w(step): c.start()
        out_buf[...] = out_acc[...].astype(BF16)
        out_cp.start()
        dx_buf[...] = dx_acc[...].astype(BF16)
        dx_cp.start()
        for g in range(NG):
            wr_kv_wait(step, g)
        for c in wr_w(step): c.wait()
        out_cp.wait()
        dx_cp.wait()


def make(unroll=3, wr=48, nocompute=False, nodma=False):
    @jax.jit
    def pallas_standalone__gqa_block_cached__near_ridge_kernel(x, k_cache, v_cache, wq, wo, grad_out):
        x2 = x.reshape(M, D)
        g2 = grad_out.reshape(M, D)
        kt = jnp.swapaxes(k_cache, 2, 3).reshape(B, H * DH, SK)
        vt = jnp.swapaxes(v_cache, 2, 3).reshape(B, H * DH, SK)
        anyspec = pl.BlockSpec(memory_space=pl.ANY)
        out, dx, dkt, dvt, dwq, dwo = pl.pallas_call(
            functools.partial(kernel, unroll=unroll, wr=wr, nocompute=nocompute),
            grid=(NSTEP,),
            in_specs=[anyspec] * 6,
            out_specs=[anyspec] * 6,
            out_shape=[jax.ShapeDtypeStruct((M, D), BF16), jax.ShapeDtypeStruct((M, D), BF16),
                       jax.ShapeDtypeStruct(kt.shape, BF16), jax.ShapeDtypeStruct(kt.shape, BF16),
                       jax.ShapeDtypeStruct(wq.shape, BF16), jax.ShapeDtypeStruct(wo.shape, BF16)],
            scratch_shapes=[pltpu.VMEM((M, D), BF16), pltpu.VMEM((M, D), BF16),
                            pltpu.VMEM((2, D, W), BF16), pltpu.VMEM((2, W, D), BF16),
                            pltpu.VMEM((2, B, W, SK), BF16), pltpu.VMEM((2, B, W, SK), BF16),
                            pltpu.VMEM((2, B, W, SK), BF16), pltpu.VMEM((2, B, W, SK), BF16),
                            pltpu.VMEM((2, D, W), BF16), pltpu.VMEM((2, W, D), BF16),
                            pltpu.VMEM((M, D), BF16), pltpu.VMEM((M, D), BF16),
                            pltpu.VMEM((M, 512), BF16), pltpu.VMEM((M, 512), BF16),
                            pltpu.VMEM((M, W), BF16), pltpu.VMEM((M, W), BF16),
                            pltpu.VMEM((HP, SQ, SK), BF16), pltpu.VMEM((HP, SQ, SK), BF16),
                            pltpu.VMEM((D, M), BF16), pltpu.VMEM((M, D), F32), pltpu.VMEM((M, D), F32),
                            pltpu.SemaphoreType.DMA((2 * NG + 2,)), pltpu.SemaphoreType.DMA((2 * NG + 2,)),
                            pltpu.SemaphoreType.DMA((4,))],
            compiler_params=pltpu.CompilerParams(dimension_semantics=("arbitrary",),
                                                 vmem_limit_bytes=110 * 1024 * 1024),
        )(x2, g2, wq, wo, kt, vt)
        unkv = lambda a: jnp.swapaxes(a.reshape(B, H, DH, SK), 2, 3)
        return (out.reshape(B, SQ, D), dx.reshape(B, SQ, D), unkv(dkt), unkv(dvt), dwq, dwo)
    return pallas_standalone__gqa_block_cached__near_ridge_kernel


pallas_standalone__gqa_block_cached__near_ridge_kernel = make()
```

```python
import contextlib
import functools
import jax
import jax.numpy as jnp
from jax import lax
import jax.experimental.pallas as pl
import jax.experimental.pallas.tpu as pltpu

B, SQ, D = 16, 64, 640
H, SK, DH = 32, 512, 192
HP = 2
W = HP * DH
M = B * SQ
NSTEP = H // HP
SCALE = DH ** -0.5
LOG2E = 1.4426950408889634
F32 = jnp.float32
BF16 = jnp.bfloat16

UB, UR = 5, 48
NRC = W // UR
NGRP = (B - 1) // UB
UPS = NGRP * NRC

S_X, S_G, S_OUT, S_DX = 0, 1, 2, 3
S_R = 4
S_WA, S_WB, S_WT = 12, 13, 14
NSEM = 15

NN = (((1,), (0,)), ((), ()))
NT = (((1,), (1,)), ((), ()))
TN = (((0,), (0,)), ((), ()))

def dot(a, b, dn):
    return lax.dot_general(a, b, dn, preferred_element_type=F32)

def pad_pair(y):
    lane = lax.broadcasted_iota(jnp.int32, (y.shape[0], 128), 1)
    mid = y[:, 128:256]
    return jnp.concatenate([y[:, 0:128], jnp.where(lane < 64, mid, 0.0), jnp.where(lane >= 64, mid, 0.0), y[:, 256:384]],
                           axis=1).astype(BF16)

def mult(v, n):
    return v if isinstance(v, int) else pl.multiple_of(v, n)

def zipl(*ls, blk=1):
    out = []
    for k in range(0, max(map(len, ls)), blk):
        for l in ls:
            out += l[k:k + blk]
    return out

def spread(big, small):
    out, j = [], 0
    for i, c in enumerate(big):
        out.append(c)
        while j < len(small) and j * len(big) <= i * len(small):
            out.append(small[j])
            j += 1
    return out + small[j:]

def kernel(x_hbm, g_hbm, wq_hbm, wo_hbm, kt_hbm, vt_hbm,
           out_hbm, dx_hbm, dkt_hbm, dvt_hbm, dwq_hbm, dwo_hbm,
           x_ref, g_ref, wq_buf, wo_buf, kt_buf, vt_buf, dkt_buf, dvt_buf, dwq_buf, dwo_buf, out_buf, dx_buf,
           q_scr, do_scr, o_scr, dq_scr, p_scr, ds_scr, xt_scr, out_acc, dx_acc,
           sem, *, nu, rtb, wt, nwp, blk, spr, prog, nocompute, scopes):
    step = pl.program_id(0)
    slot = step & 1
    last = NSTEP - 1
    scope = (lambda n: jax.named_scope(n)) if scopes else (lambda n: contextlib.nullcontext())

    def hrows(i):
        return pl.ds(mult(i * W, 128), W)

    def rd_w(i):
        s = sem.at[S_R + (i & 1) * 4]
        return [pltpu.make_async_copy(wq_hbm.at[:, hrows(i)], wq_buf.at[i & 1], s),
                pltpu.make_async_copy(wo_hbm.at[hrows(i), :], wo_buf.at[i & 1], s)]

    def rd_kv(a, i, b0, nb, s):
        src, dst = ((kt_hbm, kt_buf), (vt_hbm, vt_buf))[a]
        bs = pl.ds(b0, nb)
        return pltpu.make_async_copy(src.at[bs, hrows(i), :], dst.at[i & 1, bs], sem.at[S_R + (i & 1) * 4 + s])

    def rd_kv_main(i):
        return [rd_kv(0, i, 0, B, 1), rd_kv(1, i, 0, B - rtb, 2)]

    def rd_kv_tail(i):
        return [rd_kv(1, i, B - rtb, rtb, 3)]

    def rd_kv_first(g):
        b0, nb = (0, UB + 1) if g == 0 else (g * UB + 1, UB)
        return [rd_kv(a, 0, b0, nb, 1 + g) for a in range(2)]

    def start_r(i):
        for c in rd_w(i) + rd_kv_main(i) + rd_kv_tail(i): c.start()

    def kv_cp(a, i, bs, r, nr, s):
        src, dst = ((dkt_buf, dkt_hbm), (dvt_buf, dvt_hbm))[a]
        return pltpu.make_async_copy(src.at[i & 1, bs, pl.ds(mult(r, 16), nr), :],
                                     dst.at[bs, pl.ds(mult(i * W + r, 16), nr), :], sem.at[s])

    def unit(a, i, idx, s):
        return kv_cp(a, i, pl.ds((idx >> 3) * UB, UB), (idx & 7) * UR, UR, s)

    def punit(a, ph, k, s):
        if nu[a] == UPS:
            return unit(a, ph, k, s)
        lag = (UPS - nu[a]) * ph
        if isinstance(ph, int):
            return unit(a, ph - 1, k - lag + UPS, s) if k < lag else unit(a, ph, k - lag, s)
        if k >= (UPS - nu[a]) * (NSTEP - 2):
            return unit(a, ph, k - lag, s)
        prev = (k < lag).astype(jnp.int32)
        return unit(a, ph - prev, k - lag + UPS * prev, s)

    def b15(i, s):
        return [kv_cp(a, i, B - 1, r * UR, UR, s) for r in range(NRC) for a in range(2)]

    def dwq_piece(i, k, s, n):
        rr = pl.ds(k * (D // n), D // n)
        return pltpu.make_async_copy(dwq_buf.at[i & 1, rr, :], dwq_hbm.at[rr, hrows(i)], sem.at[s])

    def dwo_piece(i, k, s, n):
        return pltpu.make_async_copy(dwo_buf.at[i & 1, pl.ds(k * (W // n), W // n), :],
                                     dwo_hbm.at[pl.ds(mult(i * W + k * (W // n), 16), W // n), :], sem.at[s])

    def dws(i, s):
        return zipl([dwq_piece(i, k, s, nwp) for k in range(nwp)], [dwo_piece(i, k, s, nwp) for k in range(nwp)])

    def phase_a(ph):
        return spread(b15(ph - 1, S_WA), dws(ph - 1, S_WA))

    def phase_b(ph):
        return zipl(*[[punit(a, ph, k, S_WB) for k in range(nu[a] - wt[a])] for a in range(2)], blk=blk)

    def phase_t(ph):
        return zipl(*[[punit(a, ph, k, S_WT) for k in range(nu[a] - wt[a], nu[a])] for a in range(2)])

    x_cp = pltpu.make_async_copy(x_hbm, x_ref, sem.at[S_X])
    g_cp = pltpu.make_async_copy(g_hbm, g_ref, sem.at[S_G])
    out_cp = pltpu.make_async_copy(out_buf, out_hbm, sem.at[S_OUT])
    dx_cp = pltpu.make_async_copy(dx_buf, dx_hbm, sem.at[S_DX])

    def rows(b):
        return pl.ds(mult(b * SQ, SQ), SQ)

    def proj_in(sl):
        if nocompute: return
        q_scr[...] = pad_pair(dot(x_ref[...], wq_buf[sl], NN))
        do_scr[...] = pad_pair(dot(g_ref[...], wo_buf[sl], NT))

    def stage1_mm(sl, b, h):
        r = rows(b)
        s = dot(q_scr[r, h * 256:(h + 1) * 256], kt_buf[sl, b, h * 128:h * 128 + 256, :], NN)
        dp = dot(do_scr[r, h * 256:(h + 1) * 256], vt_buf[sl, b, h * 128:h * 128 + 256, :], NN)
        return s, dp

    def softmax(s, dp):
        m = jnp.max(s, axis=-1, keepdims=True)
        e = jnp.exp2((s - m) * (SCALE * LOG2E))
        l = jnp.sum(e, axis=-1, keepdims=True)
        p = e * (1.0 / l)
        delta = jnp.sum(p * dp, axis=-1, keepdims=True)
        ds = (p * (dp - delta) * SCALE).astype(BF16)
        return p.astype(BF16), ds

    def stage1_first(sl):
        if nocompute: return
        for h in range(HP):
            pb, ds = softmax(*stage1_mm(sl, 0, h))
            p_scr[h] = pb
            ds_scr[h] = ds

    def stage2(sl, b, h, pb, ds):
        r = rows(b)
        lo = 64 * h
        o = dot(pb, vt_buf[sl, b, h * 128:h * 128 + 256, :], NT)
        dq = dot(ds, kt_buf[sl, b, h * 128:h * 128 + 256, :], NT)
        o_scr[r, h * DH:(h + 1) * DH] = o[:, lo:lo + DH].astype(BF16)
        dq_scr[r, h * DH:(h + 1) * DH] = dq[:, lo:lo + DH].astype(BF16)
        dot_ = do_scr[r, h * 256:(h + 1) * 256].T[lo:lo + DH]
        qt_ = q_scr[r, h * 256:(h + 1) * 256].T[lo:lo + DH]
        dvt_buf[sl, b, h * DH:(h + 1) * DH, :] = dot(dot_, pb, NN).astype(BF16)
        dkt_buf[sl, b, h * DH:(h + 1) * DH, :] = dot(qt_, ds, NN).astype(BF16)

    def stage2_last(sl):
        if nocompute: return
        for h in range(HP):
            stage2(sl, B - 1, h, p_scr[h], ds_scr[h])

    @pl.when(step == 0)
    def _():
      with scope("prologue"):
        x_cp.start()
        g_cp.start()
        for c in rd_w(0): c.start()
        for g in range(NGRP):
            for c in rd_kv_first(g): c.start()
        start_r(1)
        out_acc[...] = jnp.zeros_like(out_acc)
        dx_acc[...] = jnp.zeros_like(dx_acc)
        x_cp.wait()
        xt_scr[...] = x_ref[...].T
        g_cp.wait()
        for c in rd_w(0): c.wait()
        proj_in(0)
        for g in range(1 if prog else NGRP):
            for c in rd_kv_first(g): c.wait()
        stage1_first(0)

    with scope("sync1"):
        @pl.when(step >= 2)
        def _():
            for c in phase_a(step - 1): c.wait()

        @pl.when(step >= 1)
        def _():
            for c in phase_b(step - 1): c.wait()
            for c in rd_kv_tail(step): c.wait()

    @pl.when(jnp.logical_and(step >= 1, step < last))
    def _():
        start_r(step + 1)

    def fin0():
        left = zipl(*[[unit(a, last - 1, k, S_WA) for k in range(UPS - (UPS - nu[a]) * last, UPS)] for a in range(2)])
        return spread(phase_a(last), left)

    def fin_units(g):
        return zipl(*[[unit(a, last, g * NRC + r, S_WB) for r in range(NRC)] for a in range(2)], blk=blk)

    @pl.when(step == last)
    def _():
        for c in fin0(): c.start()

    def body(j, c):
        for jj in range(1, NGRP):
            @pl.when(jnp.logical_and(step == last, j == jj))
            def _():
                for cp in fin_units(jj - 1): cp.start()
            if prog:
                @pl.when(jnp.logical_and(step == 0, j == jj))
                def _():
                    for cp in rd_kv_first(jj): cp.wait()
        if nocompute:
            return c
        cur = [(p_scr[h], ds_scr[h]) for h in range(HP)]
        for u in range(UB):
            b = j * UB + u
            nxt = []
            for h in range(HP):
                sdp = stage1_mm(slot, b + 1, h)
                stage2(slot, b, h, *cur[h])
                nxt.append(softmax(*sdp))
            cur = nxt
        for h in range(HP):
            p_scr[h] = cur[h][0]
            ds_scr[h] = cur[h][1]
        return c
    with scope("loop"):
        lax.fori_loop(0, NGRP, body, 0)

    @pl.when(step < last)
    def _():
        with scope("sync2"):
            for c in rd_w(step + 1) + rd_kv_main(step + 1): c.wait()
        @pl.when(step >= 1)
        def _():
            for c in phase_t(step - 1): c.wait()
            if not spr:
                for c in phase_a(step): c.start()
        if spr:
            pa = phase_a(jnp.maximum(step, 1))
            for c in spread(phase_b(step), pa):
                if any(c is q for q in pa):
                    pl.when(step >= 1)(c.start)
                else:
                    c.start()
        else:
            for c in phase_b(step): c.start()
        for c in phase_t(step): c.start()
        stage2_last(slot)
        proj_in(1 - slot)
        stage1_first(1 - slot)
        if not nocompute:
            o = o_scr[...]
            dq = dq_scr[...]
            out_acc[...] += dot(o, wo_buf[slot], NN)
            dx_acc[...] += dot(dq, wq_buf[slot], NT)
            dwo_buf[slot] = dot(o, g_ref[...], TN).astype(BF16)
            dwq_buf[slot] = dot(xt_scr[...], dq, NN).astype(BF16)

    @pl.when(step == last)
    def _():
      with scope("last"):
        sl = last % 2
        for cp in fin_units(NGRP - 1): cp.start()
        stage2_last(sl)
        for cp in b15(last, S_WB): cp.start()
        o = o_scr[...]
        dq = dq_scr[...]
        out_buf[...] = (out_acc[...] + dot(o, wo_buf[sl], NN)).astype(BF16)
        out_cp.start()
        dx_buf[...] = (dx_acc[...] + dot(dq, wq_buf[sl], NT)).astype(BF16)
        dx_cp.start()
        dwo_buf[sl] = dot(o, g_ref[...], TN).astype(BF16)
        dwo_piece(last, 0, S_X, 1).start()
        dwq_buf[sl] = dot(xt_scr[...], dq, NN).astype(BF16)
        dwq_piece(last, 0, S_G, 1).start()
        for c in phase_t(last - 1): c.wait()
        for c in fin0(): c.wait()
        for g in range(NGRP):
            for cp in fin_units(g): cp.wait()
        for cp in b15(last, S_WB): cp.wait()
        out_cp.wait()
        dx_cp.wait()
        dwo_piece(last, 0, S_X, 1).wait()
        dwq_piece(last, 0, S_G, 1).wait()


def make(nu=(24, 23), rtb=2, wt=(1, 1), nwp=4, blk=1, spr=False, prog=True, nocompute=False, nodma=False, nobc=True, nosc=False, scopes=False):
    @jax.jit
    def pallas_standalone__gqa_block_cached__near_ridge_kernel(x, k_cache, v_cache, wq, wo, grad_out):
        x2 = x.reshape(M, D)
        g2 = grad_out.reshape(M, D)
        kt = jnp.swapaxes(k_cache, 2, 3).reshape(B, H * DH, SK)
        vt = jnp.swapaxes(v_cache, 2, 3).reshape(B, H * DH, SK)
        anyspec = pl.BlockSpec(memory_space=pl.ANY)
        out, dx, dkt, dvt, dwq, dwo = pl.pallas_call(
            functools.partial(kernel, nu=nu, rtb=rtb, wt=wt, nwp=nwp, blk=blk, spr=spr, prog=prog, nocompute=nocompute, scopes=scopes),
            grid=(NSTEP,),
            in_specs=[anyspec] * 6,
            out_specs=[anyspec] * 6,
            out_shape=[jax.ShapeDtypeStruct((M, D), BF16), jax.ShapeDtypeStruct((M, D), BF16),
                       jax.ShapeDtypeStruct(kt.shape, BF16), jax.ShapeDtypeStruct(kt.shape, BF16),
                       jax.ShapeDtypeStruct(wq.shape, BF16), jax.ShapeDtypeStruct(wo.shape, BF16)],
            scratch_shapes=[pltpu.VMEM((M, D), BF16), pltpu.VMEM((M, D), BF16),
                            pltpu.VMEM((2, D, W), BF16), pltpu.VMEM((2, W, D), BF16),
                            pltpu.VMEM((2, B, W, SK), BF16), pltpu.VMEM((2, B, W, SK), BF16),
                            pltpu.VMEM((2, B, W, SK), BF16), pltpu.VMEM((2, B, W, SK), BF16),
                            pltpu.VMEM((2, D, W), BF16), pltpu.VMEM((2, W, D), BF16),
                            pltpu.VMEM((M, D), BF16), pltpu.VMEM((M, D), BF16),
                            pltpu.VMEM((M, 512), BF16), pltpu.VMEM((M, 512), BF16),
                            pltpu.VMEM((M, W), BF16), pltpu.VMEM((M, W), BF16),
                            pltpu.VMEM((HP, SQ, SK), BF16), pltpu.VMEM((HP, SQ, SK), BF16),
                            pltpu.VMEM((D, M), BF16), pltpu.VMEM((M, D), F32), pltpu.VMEM((M, D), F32),
                            pltpu.SemaphoreType.DMA((NSEM,))],
            compiler_params=pltpu.CompilerParams(dimension_semantics=("arbitrary",),
                                                 vmem_limit_bytes=110 * 1024 * 1024,
                                                 disable_bounds_checks=nobc,
                                                 disable_semaphore_checks=nosc),
        )(x2, g2, wq, wo, kt, vt)
        unkv = lambda a: jnp.swapaxes(a.reshape(B, H, DH, SK), 2, 3)
        return (out.reshape(B, SQ, D), dx.reshape(B, SQ, D), unkv(dkt), unkv(dvt), dwq, dwo)
    return pallas_standalone__gqa_block_cached__near_ridge_kernel


pallas_standalone__gqa_block_cached__near_ridge_kernel = make(blk=8)
```

```python
import jax
import jax.numpy as jnp
from jax import lax
import jax.experimental.pallas as pl
import jax.experimental.pallas.tpu as pltpu

B, SQ, D = 16, 64, 640
H, SK, DH = 32, 512, 192
HP = 2
W = HP * DH
M = B * SQ
NSTEP = H // HP
LAST = NSTEP - 1
SCALE = DH ** -0.5
LOG2E = 1.4426950408889634
F32 = jnp.float32
BF16 = jnp.bfloat16

UB, UR = 5, 48
NRC = W // UR
NGRP = (B - 1) // UB
UPS = NGRP * NRC
NU = UPS - 1
NWP = 8
RTB = 4
DU, DHD = 2, 1

S_X, S_G, S_OUT, S_DX = 0, 1, 2, 3
S_R = 4
S_WA, S_WB, S_WT = 12, 13, 14
NSEM = 15

NN = (((1,), (0,)), ((), ()))
NT = (((1,), (1,)), ((), ()))
TN = (((0,), (0,)), ((), ()))


def _dot(a, b, dn):
    return lax.dot_general(a, b, dn, preferred_element_type=F32)


def _pad_pair(y):
    lane = lax.broadcasted_iota(jnp.int32, (y.shape[0], 128), 1)
    mid = y[:, 128:256]
    return jnp.concatenate(
        [y[:, 0:128], jnp.where(lane < 64, mid, 0.0), jnp.where(lane >= 64, mid, 0.0), y[:, 256:384]],
        axis=1).astype(BF16)


def _mult(v, n):
    return v if isinstance(v, int) else pl.multiple_of(v, n)


def _zip(*lists, blk=1):
    out = []
    for k in range(0, max(map(len, lists)), blk):
        for lst in lists:
            out += lst[k:k + blk]
    return out


def _start(copies):
    for c in copies:
        c.start()


def _wait(copies):
    for c in copies:
        c.wait()


def _kernel(x_hbm, g_hbm, wq_hbm, wo_hbm, kt_hbm, vt_hbm,
            out_hbm, dx_hbm, dkt_hbm, dvt_hbm, dwq_hbm, dwo_hbm,
            x_ref, g_ref, wq_buf, wo_buf, kt_buf, vt_buf, dkt_buf, dvt_buf, dwq_buf, dwo_buf,
            out_buf, dx_buf, q_scr, do_scr, o_scr, dq_scr, p_scr, ds_scr, pdef_scr, xt_scr,
            out_acc, dx_acc, sem):
    step = pl.program_id(0)
    slot = step & 1
    copy = pltpu.make_async_copy

    def hrows(i):
        return pl.ds(_mult(i * W, 128), W)

    def rd_w(i):
        s = sem.at[S_R + (i & 1) * 4]
        return [copy(wq_hbm.at[:, hrows(i)], wq_buf.at[i & 1], s),
                copy(wo_hbm.at[hrows(i), :], wo_buf.at[i & 1], s)]

    def rd_kv(a, i, b0, nb, s):
        src, dst = ((kt_hbm, kt_buf), (vt_hbm, vt_buf))[a]
        bs = pl.ds(b0, nb)
        return copy(src.at[bs, hrows(i), :], dst.at[i & 1, bs], sem.at[S_R + (i & 1) * 4 + s])

    def rd_main(i):
        return rd_w(i) + [rd_kv(0, i, 0, B, 1), rd_kv(1, i, 0, B - RTB, 2)]

    def rd_tail(i):
        return [rd_kv(1, i, B - RTB, RTB, 3)]

    def rd_first(g):
        b0, nb = (0, UB + 1) if g == 0 else (g * UB + 1, UB)
        return [rd_kv(a, 0, b0, nb, 1 + g) for a in range(2)]

    def wr_kv(a, i, bs, r, s):
        src, dst = ((dkt_buf, dkt_hbm), (dvt_buf, dvt_hbm))[a]
        return copy(src.at[i & 1, bs, pl.ds(_mult(r, 16), UR), :],
                    dst.at[bs, pl.ds(_mult(i * W + r, 16), UR), :], sem.at[s])

    def unit(a, i, idx, s):
        return wr_kv(a, i, pl.ds((idx >> 3) * UB, UB), (idx & 7) * UR, s)

    def phase_unit(a, ph, k, s):
        if isinstance(ph, int):
            return unit(a, ph - 1, k - ph + UPS, s) if k < ph else unit(a, ph, k - ph, s)
        if k >= LAST - 1:
            return unit(a, ph, k - ph, s)
        prev = (k < ph).astype(jnp.int32)
        return unit(a, ph - prev, k - ph + UPS * prev, s)

    def wr_b15(i, s):
        return [wr_kv(a, i, B - 1, r * UR, s) for r in range(NRC) for a in range(2)]

    def wr_dwq(i, s, n):
        return [copy(dwq_buf.at[i & 1, pl.ds(k * (D // n), D // n), :],
                     dwq_hbm.at[pl.ds(k * (D // n), D // n), hrows(i)], sem.at[s]) for k in range(n)]

    def wr_dwo(i, s, n):
        return [copy(dwo_buf.at[i & 1, pl.ds(k * (W // n), W // n), :],
                     dwo_hbm.at[pl.ds(_mult(i * W + k * (W // n), 16), W // n), :], sem.at[s])
                for k in range(n)]

    def phase_a(ph):
        return _zip(wr_b15(ph - 1, S_WA), _zip(wr_dwq(ph - 1, S_WA, NWP), wr_dwo(ph - 1, S_WA, NWP)))

    def phase_b(ph):
        return _zip([phase_unit(0, ph, k, S_WB) for k in range(NU)],
                    [phase_unit(1, ph, k, S_WB) for k in range(NU - 1)], blk=NRC)

    def phase_t(ph):
        return [phase_unit(1, ph, NU - 1, S_WT)]

    def final_left():
        left = _zip(*[[unit(a, LAST - 1, k, S_WA) for k in range(UPS - LAST, UPS)] for a in range(2)])
        return _zip(phase_a(LAST), left)

    def final_group(g):
        return [unit(a, LAST, g * NRC + r, S_WB) for a in range(2) for r in range(NRC)]

    def rows(b):
        return pl.ds(_mult(b * SQ, SQ), SQ)

    def proj_in(sl):
        q_scr[...] = _pad_pair(_dot(x_ref[...], wq_buf[sl], NN))
        do_scr[...] = _pad_pair(_dot(g_ref[...], wo_buf[sl], NT))

    def scores(sl, b, h):
        r = rows(b)
        s = _dot(q_scr[r, h * 256:(h + 1) * 256], kt_buf[sl, b, h * 128:h * 128 + 256, :], NN)
        dp = _dot(do_scr[r, h * 256:(h + 1) * 256], vt_buf[sl, b, h * 128:h * 128 + 256, :], NN)
        return s, dp

    def softmax_fwd_bwd(s, dp):
        m = jnp.max(s, axis=-1, keepdims=True)
        e = jnp.exp2((s - m) * (SCALE * LOG2E))
        p = e * (1.0 / jnp.sum(e, axis=-1, keepdims=True))
        delta = jnp.sum(p * dp, axis=-1, keepdims=True)
        ds = p * (dp - delta) * SCALE
        return p.astype(BF16), ds.astype(BF16)

    def first_scores(sl):
        for h in range(HP):
            p_scr[h], ds_scr[h] = softmax_fwd_bwd(*scores(sl, 0, h))

    def attn_out(sl, b, h, p):
        o = _dot(p, vt_buf[sl, b, h * 128:h * 128 + 256, :], NT)
        o_scr[rows(b), h * DH:(h + 1) * DH] = o[:, 64 * h:64 * h + DH].astype(BF16)

    def attn_grads(sl, b, h, p, ds):
        r = rows(b)
        lo = 64 * h
        dq = _dot(ds, kt_buf[sl, b, h * 128:h * 128 + 256, :], NT)
        dq_scr[r, h * DH:(h + 1) * DH] = dq[:, lo:lo + DH].astype(BF16)
        do_t = do_scr[r, h * 256:(h + 1) * 256].T[lo:lo + DH]
        q_t = q_scr[r, h * 256:(h + 1) * 256].T[lo:lo + DH]
        dvt_buf[sl, b, h * DH:(h + 1) * DH, :] = _dot(do_t, p, NN).astype(BF16)
        dkt_buf[sl, b, h * DH:(h + 1) * DH, :] = _dot(q_t, ds, NN).astype(BF16)

    def finish_attention(sl):
        for h in range(HP):
            attn_out(sl, B - 1, h, p_scr[h])
            attn_grads(sl, B - 1, h, p_scr[h], ds_scr[h])
        for j in range(NGRP):
            attn_out(sl, j * UB + DU, DHD, pdef_scr[j])

    @pl.when(step == 0)
    def _():
        x_cp = copy(x_hbm, x_ref, sem.at[S_X])
        g_cp = copy(g_hbm, g_ref, sem.at[S_G])
        _start([x_cp, g_cp] + rd_w(0))
        for g in range(NGRP):
            _start(rd_first(g))
        _start(rd_main(1) + rd_tail(1))
        out_acc[...] = jnp.zeros_like(out_acc)
        dx_acc[...] = jnp.zeros_like(dx_acc)
        x_cp.wait()
        xt_scr[...] = x_ref[...].T
        g_cp.wait()
        _wait(rd_w(0))
        proj_in(0)
        _wait(rd_first(0))
        first_scores(0)

    @pl.when(step >= 2)
    def _():
        _wait(phase_a(step - 1))

    @pl.when(step >= 1)
    def _():
        _wait(phase_b(step - 1))
        _wait(rd_tail(step))

    @pl.when(jnp.logical_and(step >= 1, step < LAST))
    def _():
        _start(rd_main(step + 1) + rd_tail(step + 1))

    @pl.when(step == LAST)
    def _():
        _start(final_left())

    def body(j, carry):
        @pl.when(jnp.logical_and(j > 0, jnp.logical_or(step == 0, step == LAST)))
        def _():
            @pl.when(step == LAST)
            def _():
                _start(final_group(j - 1))

            for g in range(1, NGRP):
                @pl.when(jnp.logical_and(step == 0, j == g))
                def _():
                    _wait(rd_first(g))

        cur = [(p_scr[h], ds_scr[h]) for h in range(HP)]
        for u in range(UB):
            b = j * UB + u
            nxt = []
            for h in range(HP):
                s_dp = scores(slot, b + 1, h)
                p, ds = cur[h]
                if (u, h) == (DU, DHD):
                    pdef_scr[j] = p
                else:
                    attn_out(slot, b, h, p)
                attn_grads(slot, b, h, p, ds)
                nxt.append(softmax_fwd_bwd(*s_dp))
            cur = nxt
        for h in range(HP):
            p_scr[h], ds_scr[h] = cur[h]
        return carry

    lax.fori_loop(0, NGRP, body, 0)

    @pl.when(step < LAST)
    def _():
        _wait(rd_main(step + 1))

        @pl.when(step >= 1)
        def _():
            _wait(phase_t(step - 1))
            _start(phase_a(step))

        _start(phase_b(step) + phase_t(step))
        finish_attention(slot)
        proj_in(1 - slot)
        first_scores(1 - slot)
        o = o_scr[...]
        dq = dq_scr[...]
        out_acc[...] += _dot(o, wo_buf[slot], NN)
        dx_acc[...] += _dot(dq, wq_buf[slot], NT)
        dwo_buf[slot] = _dot(o, g_ref[...], TN).astype(BF16)
        dwq_buf[slot] = _dot(xt_scr[...], dq, NN).astype(BF16)

    @pl.when(step == LAST)
    def _():
        sl = LAST & 1
        out_cp = copy(out_buf, out_hbm, sem.at[S_OUT])
        dx_cp = copy(dx_buf, dx_hbm, sem.at[S_DX])
        _start(final_group(NGRP - 1))
        finish_attention(sl)
        _start(wr_b15(LAST, S_WB))
        o = o_scr[...]
        dq = dq_scr[...]
        out_buf[...] = (out_acc[...] + _dot(o, wo_buf[sl], NN)).astype(BF16)
        out_cp.start()
        dx_buf[...] = (dx_acc[...] + _dot(dq, wq_buf[sl], NT)).astype(BF16)
        dx_cp.start()
        dwo_buf[sl] = _dot(o, g_ref[...], TN).astype(BF16)
        _start(wr_dwo(LAST, S_X, 1))
        dwq_buf[sl] = _dot(xt_scr[...], dq, NN).astype(BF16)
        _start(wr_dwq(LAST, S_G, 1))
        _wait(phase_t(LAST - 1))
        _wait(final_left())
        for g in range(NGRP):
            _wait(final_group(g))
        _wait(wr_b15(LAST, S_WB))
        _wait([out_cp, dx_cp] + wr_dwo(LAST, S_X, 1) + wr_dwq(LAST, S_G, 1))


@jax.jit
def pallas_standalone__gqa_block_cached__near_ridge_kernel(
    x: jax.Array,
    k_cache: jax.Array,
    v_cache: jax.Array,
    wq: jax.Array,
    wo: jax.Array,
    grad_out: jax.Array,
):
    kt = jnp.swapaxes(k_cache, 2, 3).reshape(B, H * DH, SK)
    vt = jnp.swapaxes(v_cache, 2, 3).reshape(B, H * DH, SK)
    hbm = pl.BlockSpec(memory_space=pl.ANY)
    vmem = pltpu.VMEM
    out, dx, dkt, dvt, dwq, dwo = pl.pallas_call(
        _kernel,
        grid=(NSTEP,),
        in_specs=[hbm] * 6,
        out_specs=[hbm] * 6,
        out_shape=[
            jax.ShapeDtypeStruct((M, D), BF16), jax.ShapeDtypeStruct((M, D), BF16),
            jax.ShapeDtypeStruct(kt.shape, BF16), jax.ShapeDtypeStruct(kt.shape, BF16),
            jax.ShapeDtypeStruct(wq.shape, BF16), jax.ShapeDtypeStruct(wo.shape, BF16),
        ],
        scratch_shapes=[
            vmem((M, D), BF16), vmem((M, D), BF16),
            vmem((2, D, W), BF16), vmem((2, W, D), BF16),
            vmem((2, B, W, SK), BF16), vmem((2, B, W, SK), BF16),
            vmem((2, B, W, SK), BF16), vmem((2, B, W, SK), BF16),
            vmem((2, D, W), BF16), vmem((2, W, D), BF16),
            vmem((M, D), BF16), vmem((M, D), BF16),
            vmem((M, 512), BF16), vmem((M, 512), BF16),
            vmem((M, W), BF16), vmem((M, W), BF16),
            vmem((HP, SQ, SK), BF16), vmem((HP, SQ, SK), BF16),
            vmem((NGRP, SQ, SK), BF16),
            vmem((D, M), BF16),
            vmem((M, D), F32), vmem((M, D), F32),
            pltpu.SemaphoreType.DMA((NSEM,)),
        ],
        compiler_params=pltpu.CompilerParams(
            dimension_semantics=("arbitrary",),
            vmem_limit_bytes=100 * 1024 * 1024,
            disable_bounds_checks=True,
            disable_semaphore_checks=True,
        ),
    )(x.reshape(M, D), grad_out.reshape(M, D), wq, wo, kt, vt)

    def un_t(a):
        return jnp.swapaxes(a.reshape(B, H, DH, SK), 2, 3)

    return (out.reshape(B, SQ, D), dx.reshape(B, SQ, D), un_t(dkt), un_t(dvt), dwq, dwo)
```

```python
import jax
import jax.numpy as jnp
from jax import lax
import jax.experimental.pallas as pl
import jax.experimental.pallas.tpu as pltpu

B, SQ, D = 16, 64, 640
H, SK, DH = 32, 512, 192
HP = 2
W = HP * DH
M = B * SQ
NSTEP = H // HP
LAST = NSTEP - 1
SCALE = DH ** -0.5
LOG2E = 1.4426950408889634
F32 = jnp.float32
BF16 = jnp.bfloat16

UB, UR = 5, 48
NRC = W // UR
NGRP = (B - 1) // UB
UPS = NGRP * NRC
NU = UPS - 1
NWP = 8
RTB = 4
DU, DHD = 2, 1

S_X, S_G, S_OUT, S_DX = 0, 1, 2, 3
S_R = 4
S_WA, S_WB, S_WT = 12, 13, 14
NSEM = 15

NN = (((1,), (0,)), ((), ()))
NT = (((1,), (1,)), ((), ()))
TN = (((0,), (0,)), ((), ()))


def _dot(a, b, dn):
    return lax.dot_general(a, b, dn, preferred_element_type=F32)


def _pad_pair(y):
    lane = lax.broadcasted_iota(jnp.int32, (y.shape[0], 128), 1)
    mid = y[:, 128:256]
    return jnp.concatenate(
        [y[:, 0:128], jnp.where(lane < 64, mid, 0.0), jnp.where(lane >= 64, mid, 0.0), y[:, 256:384]],
        axis=1).astype(BF16)


def _mult(v, n):
    return v if isinstance(v, int) else pl.multiple_of(v, n)


def _zip(*lists, blk=1):
    out = []
    for k in range(0, max(map(len, lists)), blk):
        for lst in lists:
            out += lst[k:k + blk]
    return out


def _start(copies):
    for c in copies:
        c.start()


def _wait(copies):
    for c in copies:
        c.wait()


def _kernel(x_hbm, g_hbm, wq_hbm, wo_hbm, kt_hbm, vt_hbm,
            out_hbm, dx_hbm, dkt_hbm, dvt_hbm, dwq_hbm, dwo_hbm,
            x_ref, g_ref, wq_buf, wo_buf, kt_buf, vt_buf, dkt_buf, dvt_buf, dwq_buf, dwo_buf,
            out_buf, dx_buf, q_scr, do_scr, o_scr, dq_scr, p_scr, ds_scr, pdef_scr, xt_scr,
            out_acc, dx_acc, sem):
    step = pl.program_id(0)
    slot = step & 1
    copy = pltpu.make_async_copy

    def hrows(i):
        return pl.ds(_mult(i * W, 128), W)

    def rd_w(i):
        s = sem.at[S_R + (i & 1) * 4]
        return [copy(wq_hbm.at[:, hrows(i)], wq_buf.at[i & 1], s),
                copy(wo_hbm.at[hrows(i), :], wo_buf.at[i & 1], s)]

    def rd_kv(a, i, b0, nb, s):
        src, dst = ((kt_hbm, kt_buf), (vt_hbm, vt_buf))[a]
        bs = pl.ds(b0, nb)
        return copy(src.at[bs, hrows(i), :], dst.at[i & 1, bs], sem.at[S_R + (i & 1) * 4 + s])

    def rd_main(i):
        return rd_w(i) + [rd_kv(0, i, 0, B, 1), rd_kv(1, i, 0, B - RTB, 2)]

    def rd_tail(i):
        return [rd_kv(1, i, B - RTB, RTB, 3)]

    def rd_first(g):
        b0, nb = (0, UB + 1) if g == 0 else (g * UB + 1, UB)
        return [rd_kv(a, 0, b0, nb, 1 + g) for a in range(2)]

    def wr_kv(a, i, bs, r, s):
        src, dst = ((dkt_buf, dkt_hbm), (dvt_buf, dvt_hbm))[a]
        return copy(src.at[i & 1, bs, pl.ds(_mult(r, 16), UR), :],
                    dst.at[bs, pl.ds(_mult(i * W + r, 16), UR), :], sem.at[s])

    def unit(a, i, idx, s):
        return wr_kv(a, i, pl.ds((idx >> 3) * UB, UB), (idx & 7) * UR, s)

    def phase_unit(a, ph, k, s):
        if isinstance(ph, int):
            return unit(a, ph - 1, k - ph + UPS, s) if k < ph else unit(a, ph, k - ph, s)
        if k >= LAST - 1:
            return unit(a, ph, k - ph, s)
        prev = (k < ph).astype(jnp.int32)
        return unit(a, ph - prev, k - ph + UPS * prev, s)

    def wr_b15(i, s):
        return [wr_kv(a, i, B - 1, r * UR, s) for r in range(NRC) for a in range(2)]

    def wr_dwq(i, s, n=NWP):
        return [copy(dwq_buf.at[i & 1, pl.ds(k * (D // n), D // n), :],
                     dwq_hbm.at[pl.ds(k * (D // n), D // n), hrows(i)], sem.at[s]) for k in range(n)]

    def wr_dwo(i, s, n=NWP):
        return [copy(dwo_buf.at[i & 1, pl.ds(k * (W // n), W // n), :],
                     dwo_hbm.at[pl.ds(_mult(i * W + k * (W // n), 16), W // n), :], sem.at[s])
                for k in range(n)]

    def wr_act(buf, dst, s):
        return [copy(buf.at[pl.ds(b * SQ, SQ), :], dst.at[pl.ds(b * SQ, SQ), :], sem.at[s]) for b in range(B)]

    def phase_a(ph):
        return _zip(wr_b15(ph - 1, S_WA), _zip(wr_dwq(ph - 1, S_WA), wr_dwo(ph - 1, S_WA)))

    def phase_b(ph):
        return _zip([phase_unit(0, ph, k, S_WB) for k in range(NU)],
                    [phase_unit(1, ph, k, S_WB) for k in range(NU - 1)], blk=NRC)

    def phase_t(ph):
        return [phase_unit(1, ph, NU - 1, S_WT)]

    def final_left():
        left = _zip(*[[unit(a, LAST - 1, k, S_WA) for k in range(UPS - LAST, UPS)] for a in range(2)])
        return _zip(phase_a(LAST), left)

    def final_group(g):
        return [unit(a, LAST, g * NRC + r, S_WB) for a in range(2) for r in range(NRC)]

    def rows(b):
        return pl.ds(_mult(b * SQ, SQ), SQ)

    def proj_in(sl):
        q_scr[...] = _pad_pair(_dot(x_ref[...], wq_buf[sl], NN))
        do_scr[...] = _pad_pair(_dot(g_ref[...], wo_buf[sl], NT))

    def scores(sl, b, h):
        r = rows(b)
        s = _dot(q_scr[r, h * 256:(h + 1) * 256], kt_buf[sl, b, h * 128:h * 128 + 256, :], NN)
        dp = _dot(do_scr[r, h * 256:(h + 1) * 256], vt_buf[sl, b, h * 128:h * 128 + 256, :], NN)
        return s, dp

    def softmax_fwd_bwd(s, dp):
        m = jnp.max(s, axis=-1, keepdims=True)
        e = jnp.exp2((s - m) * (SCALE * LOG2E))
        p = e * (1.0 / jnp.sum(e, axis=-1, keepdims=True))
        delta = jnp.sum(p * dp, axis=-1, keepdims=True)
        ds = p * (dp - delta) * SCALE
        return p.astype(BF16), ds.astype(BF16)

    def first_scores(sl):
        for h in range(HP):
            p_scr[h], ds_scr[h] = softmax_fwd_bwd(*scores(sl, 0, h))

    def attn_out(sl, b, h, p):
        o = _dot(p, vt_buf[sl, b, h * 128:h * 128 + 256, :], NT)
        o_scr[rows(b), h * DH:(h + 1) * DH] = o[:, 64 * h:64 * h + DH].astype(BF16)

    def attn_grads(sl, b, h, p, ds):
        r = rows(b)
        lo = 64 * h
        dq = _dot(ds, kt_buf[sl, b, h * 128:h * 128 + 256, :], NT)
        dq_scr[r, h * DH:(h + 1) * DH] = dq[:, lo:lo + DH].astype(BF16)
        do_t = do_scr[r, h * 256:(h + 1) * 256].T[lo:lo + DH]
        q_t = q_scr[r, h * 256:(h + 1) * 256].T[lo:lo + DH]
        dvt_buf[sl, b, h * DH:(h + 1) * DH, :] = _dot(do_t, p, NN).astype(BF16)
        dkt_buf[sl, b, h * DH:(h + 1) * DH, :] = _dot(q_t, ds, NN).astype(BF16)

    def finish_attention(sl):
        for h in range(HP):
            attn_out(sl, B - 1, h, p_scr[h])
            attn_grads(sl, B - 1, h, p_scr[h], ds_scr[h])
        for j in range(NGRP):
            attn_out(sl, j * UB + DU, DHD, pdef_scr[j])

    @pl.when(step == 0)
    def _():
        x_cp = copy(x_hbm, x_ref, sem.at[S_X])
        g_cp = copy(g_hbm, g_ref, sem.at[S_G])
        _start([x_cp, g_cp] + rd_w(0))
        for g in range(NGRP):
            _start(rd_first(g))
        _start(rd_main(1) + rd_tail(1))
        out_acc[...] = jnp.zeros_like(out_acc)
        dx_acc[...] = jnp.zeros_like(dx_acc)
        x_cp.wait()
        xt_scr[...] = x_ref[...].T
        g_cp.wait()
        _wait(rd_w(0))
        proj_in(0)
        _wait(rd_first(0))
        first_scores(0)

    @pl.when(step >= 2)
    def _():
        _wait(phase_a(step - 1))

    @pl.when(step >= 1)
    def _():
        _wait(phase_b(step - 1))
        _wait(rd_tail(step))

    @pl.when(jnp.logical_and(step >= 1, step < LAST))
    def _():
        _start(rd_main(step + 1) + rd_tail(step + 1))

    @pl.when(step == LAST)
    def _():
        _start(final_left())

    def body(j, carry):
        @pl.when(jnp.logical_and(j > 0, jnp.logical_or(step == 0, step == LAST)))
        def _():
            @pl.when(step == LAST)
            def _():
                _start(final_group(j - 1))

            for g in range(1, NGRP):
                @pl.when(jnp.logical_and(step == 0, j == g))
                def _():
                    _wait(rd_first(g))

        cur = [(p_scr[h], ds_scr[h]) for h in range(HP)]
        for u in range(UB):
            b = j * UB + u
            nxt = []
            for h in range(HP):
                s_dp = scores(slot, b + 1, h)
                p, ds = cur[h]
                if (u, h) == (DU, DHD):
                    pdef_scr[j] = p
                else:
                    attn_out(slot, b, h, p)
                attn_grads(slot, b, h, p, ds)
                nxt.append(softmax_fwd_bwd(*s_dp))
            cur = nxt
        for h in range(HP):
            p_scr[h], ds_scr[h] = cur[h]
        return carry

    lax.fori_loop(0, NGRP, body, 0)

    @pl.when(step < LAST)
    def _():
        _wait(rd_main(step + 1))

        @pl.when(step >= 1)
        def _():
            _wait(phase_t(step - 1))
            _start(phase_a(step))

        _start(phase_b(step) + phase_t(step))
        finish_attention(slot)
        proj_in(1 - slot)
        first_scores(1 - slot)
        o = o_scr[...]
        dq = dq_scr[...]
        out_acc[...] += _dot(o, wo_buf[slot], NN)
        dx_acc[...] += _dot(dq, wq_buf[slot], NT)
        dwo_buf[slot] = _dot(o, g_ref[...], TN).astype(BF16)
        dwq_buf[slot] = _dot(xt_scr[...], dq, NN).astype(BF16)

    @pl.when(step == LAST)
    def _():
        sl = LAST & 1
        acts = _zip(wr_act(out_buf, out_hbm, S_OUT), wr_act(dx_buf, dx_hbm, S_DX), wr_b15(LAST, S_WB))
        dws = _zip(wr_dwo(LAST, S_X), wr_dwq(LAST, S_G))
        _start(final_group(NGRP - 1))
        finish_attention(sl)
        o = o_scr[...]
        dq = dq_scr[...]
        out_buf[...] = (out_acc[...] + _dot(o, wo_buf[sl], NN)).astype(BF16)
        dx_buf[...] = (dx_acc[...] + _dot(dq, wq_buf[sl], NT)).astype(BF16)
        _start(acts)
        dwo_buf[sl] = _dot(o, g_ref[...], TN).astype(BF16)
        dwq_buf[sl] = _dot(xt_scr[...], dq, NN).astype(BF16)
        _start(dws)
        _wait(phase_t(LAST - 1))
        _wait(final_left())
        for g in range(NGRP):
            _wait(final_group(g))
        _wait(acts + dws)


@jax.jit
def pallas_standalone__gqa_block_cached__near_ridge_kernel(
    x: jax.Array,
    k_cache: jax.Array,
    v_cache: jax.Array,
    wq: jax.Array,
    wo: jax.Array,
    grad_out: jax.Array,
):
    kt = jnp.swapaxes(k_cache, 2, 3).reshape(B, H * DH, SK)
    vt = jnp.swapaxes(v_cache, 2, 3).reshape(B, H * DH, SK)
    hbm = pl.BlockSpec(memory_space=pl.ANY)
    vmem = pltpu.VMEM
    out, dx, dkt, dvt, dwq, dwo = pl.pallas_call(
        _kernel,
        grid=(NSTEP,),
        in_specs=[hbm] * 6,
        out_specs=[hbm] * 6,
        out_shape=[
            jax.ShapeDtypeStruct((M, D), BF16), jax.ShapeDtypeStruct((M, D), BF16),
            jax.ShapeDtypeStruct(kt.shape, BF16), jax.ShapeDtypeStruct(kt.shape, BF16),
            jax.ShapeDtypeStruct(wq.shape, BF16), jax.ShapeDtypeStruct(wo.shape, BF16),
        ],
        scratch_shapes=[
            vmem((M, D), BF16), vmem((M, D), BF16),
            vmem((2, D, W), BF16), vmem((2, W, D), BF16),
            vmem((2, B, W, SK), BF16), vmem((2, B, W, SK), BF16),
            vmem((2, B, W, SK), BF16), vmem((2, B, W, SK), BF16),
            vmem((2, D, W), BF16), vmem((2, W, D), BF16),
            vmem((M, D), BF16), vmem((M, D), BF16),
            vmem((M, 512), BF16), vmem((M, 512), BF16),
            vmem((M, W), BF16), vmem((M, W), BF16),
            vmem((HP, SQ, SK), BF16), vmem((HP, SQ, SK), BF16),
            vmem((NGRP, SQ, SK), BF16),
            vmem((D, M), BF16),
            vmem((M, D), F32), vmem((M, D), F32),
            pltpu.SemaphoreType.DMA((NSEM,)),
        ],
        compiler_params=pltpu.CompilerParams(
            dimension_semantics=("arbitrary",),
            vmem_limit_bytes=100 * 1024 * 1024,
            disable_bounds_checks=True,
            disable_semaphore_checks=True,
        ),
    )(x.reshape(M, D), grad_out.reshape(M, D), wq, wo, kt, vt)

    def un_t(a):
        return jnp.swapaxes(a.reshape(B, H, DH, SK), 2, 3)

    return (out.reshape(B, SQ, D), dx.reshape(B, SQ, D), un_t(dkt), un_t(dvt), dwq, dwo)
```
